```python
import os as _os
_os.environ.setdefault("JAX_PLATFORMS", "cpu")
import jax
import jax.numpy as jnp

def _softmax(x, axis=-1):
    return jax.nn.softmax(x, axis=axis)
def _gelu(x):
    return jax.nn.gelu(x, approximate=True)
def _silu(x):
    return jax.nn.silu(x)
def _sigmoid(x):
    return jax.nn.sigmoid(x)
def _layernorm(x, axis=-1, eps=1e-5):
    m = jnp.mean(x, axis=axis, keepdims=True)
    v = jnp.var(x, axis=axis, keepdims=True)
    return (x - m) / jnp.sqrt(v + eps)
def _scatter_add(tgt, idx, src, axis=0):
    return tgt.at[idx].add(src)
def _segment_sum(src, seg, n):
    return jax.ops.segment_sum(src, seg, n)
class _Rng:
    def __init__(self, key):
        self._k = key
    def _next(self):
        self._k, sub = jax.random.split(self._k)
        return sub
    def normal(self, shape):
        return jax.random.normal(self._next(), shape, dtype=jnp.bfloat16)
    def randint(self, lo, hi, shape):
        return jax.random.randint(self._next(), shape, lo, hi, dtype=jnp.int32)
    def uniform(self, shape, lo=0.0, hi=1.0):
        return jax.random.uniform(self._next(), shape, jnp.bfloat16, lo, hi)
    def permutation(self, n):
        return jax.random.permutation(self._next(), n)


kernel_name = 'standalone__mha_softmax__near_ridge'

def setup_inputs():
    _rng = _Rng(jax.random.key(int.from_bytes(__import__("os").urandom(4), "little")))
    _w = (lambda a: (lambda t: t.astype(jnp.bfloat16) if jnp.issubdtype(t.dtype, jnp.floating) else t)(jnp.asarray(a)))
    B, H, Sq, Sk, D = 32, 32, 288, 512, 128
    return {
        "q": _w((lambda *s: _rng.normal(s) * 0.4)(B, H, Sq, D)),
        "k": _w((lambda *s: _rng.normal(s) * 0.4)(B, H, Sk, D)),
        "v": _w((lambda *s: _rng.normal(s) * 0.05)(B, H, Sk, D)),
    }

def reference(q, k, v):
    scale = q.shape[-1] ** -0.5
    scores = jnp.einsum("bhqd,bhkd->bhqk", q, k) * scale
    p = _softmax(scores, axis=-1)
    return jnp.einsum("bhqk,bhkd->bhqd", p, v)
```

```python
import jax
import jax.numpy as jnp
import jax.experimental.pallas as pl
import jax.experimental.pallas.tpu as pltpu

_LOG2E = 1.4426950408889634


@jax.jit
def pallas_standalone__mha_softmax__near_ridge_kernel(
    q: jax.Array,
    k: jax.Array,
    v: jax.Array,
):
    B, H, Sq, D = q.shape
    Sk = k.shape[2]
    BH = B * H
    HB = 16
    c = (D ** -0.5) * _LOG2E

    q3 = q.reshape(BH, Sq, D)
    k3 = k.reshape(BH, Sk, D)
    v3 = v.reshape(BH, Sk, D)

    def kernel_function(q_ref, k_ref, v_ref, o_ref):
        def body(h, carry):
            s = jax.lax.dot_general(
                q_ref[h], k_ref[h], (((1,), (1,)), ((), ())),
                preferred_element_type=jnp.float32)
            m = jnp.max(s, axis=-1, keepdims=True)
            p = jnp.exp2((s - m) * c)
            l = jnp.sum(p, axis=-1, keepdims=True)
            o = jnp.dot(p.astype(jnp.bfloat16), v_ref[h],
                        preferred_element_type=jnp.float32)
            o_ref[h] = (o / l).astype(o_ref.dtype)
            return carry

        jax.lax.fori_loop(0, HB, body, 0, unroll=2)

    out = pl.pallas_call(
        kernel_function,
        grid=(BH // HB,),
        in_specs=[
            pl.BlockSpec((HB, Sq, D), lambda i: (i, 0, 0)),
            pl.BlockSpec((HB, Sk, D), lambda i: (i, 0, 0)),
            pl.BlockSpec((HB, Sk, D), lambda i: (i, 0, 0)),
        ],
        out_specs=pl.BlockSpec((HB, Sq, D), lambda i: (i, 0, 0)),
        out_shape=jax.ShapeDtypeStruct((BH, Sq, D), q.dtype),
        compiler_params=pltpu.CompilerParams(
            dimension_semantics=("arbitrary",),
            vmem_limit_bytes=100 * 1024 * 1024,
        ),
    )(q3, k3, v3)
    return out.reshape(B, H, Sq, D)
```

```python
import jax
import jax.numpy as jnp
import jax.experimental.pallas as pl
import jax.experimental.pallas.tpu as pltpu

_LOG2E = 1.4426950408889634

_C = 8
_R = 8
_WR = 128
_WS = 16


@jax.jit
def pallas_standalone__mha_softmax__near_ridge_kernel(
    q: jax.Array,
    k: jax.Array,
    v: jax.Array,
):
    B, H, Sq, D = q.shape
    Sk = k.shape[2]
    BH = B * H
    C, R, WR, WS = _C, _R, _WR, _WS
    N = BH // C
    W0 = N - R
    G = BH * Sq // (WR * WS)
    GA = (W0 * C * Sq) // (WR * WS)
    assert BH % C == 0 and (BH * Sq) % (WR * WS) == 0 and Sq % 16 == 0
    c = (D ** -0.5) * _LOG2E

    def head(qh, kh, vh):
        s = jax.lax.dot_general(qh, kh, (((1,), (1,)), ((), ())),
                                preferred_element_type=jnp.float32)
        m = jnp.max(s, axis=-1, keepdims=True)
        p = jnp.exp2((s - m) * c)
        l = jnp.sum(p, axis=-1, keepdims=True)
        o = jnp.dot(p.astype(jnp.bfloat16), vh,
                    preferred_element_type=jnp.float32)
        return o / l

    def kernel_function(q_hbm, k_hbm, v_hbm, o_hbm, qb, kb, vb, ob, sin, sout):
        ob4 = ob.reshape(G, WS, WR, D)

        def in_copies(i, slot):
            return [
                pltpu.make_async_copy(src.at[pl.ds(i * C, C)], dst.at[slot],
                                      sin.at[slot * 3 + j])
                for j, (src, dst) in enumerate(
                    ((q_hbm, qb), (k_hbm, kb), (v_hbm, vb)))
            ]

        def out_copies(g0, g1):
            return [
                pltpu.make_async_copy(ob4.at[pl.ds(g0, g1 - g0), s],
                                      o_hbm.at[pl.ds(g0, g1 - g0), s],
                                      sout.at[0])
                for s in range(WS)
            ]

        for j in range(R - 1):
            for cp in in_copies(j, j):
                cp.start()

        def step(i, carry):
            slot = i % R

            @pl.when(i <= W0)
            def _():
                nxt = i + R - 1
                for cp in in_copies(nxt, nxt % R):
                    cp.start()

            @pl.when(jnp.logical_or(i < W0, i == N - 1))
            def _():
                for cp in in_copies(i, slot):
                    cp.wait()

            @pl.when(i == W0)
            def _():
                for j in range(W0, N - 1):
                    for cp in in_copies(j, j % R):
                        cp.wait()
                for cp in out_copies(0, GA):
                    cp.start()

            def per_head(h, cc):
                row0 = pl.multiple_of((i * C + h) * Sq, 16)
                ob[pl.ds(row0, Sq), :] = head(
                    qb[slot, h], kb[slot, h], vb[slot, h]).astype(ob.dtype)
                return cc

            jax.lax.fori_loop(0, C, per_head, 0, unroll=True)
            return carry

        jax.lax.fori_loop(0, N, step, 0)
        for cp in out_copies(GA, G):
            cp.start()
        for cp in out_copies(0, GA):
            cp.wait()
        for cp in out_copies(GA, G):
            cp.wait()

    out = pl.pallas_call(
        kernel_function,
        in_specs=[pl.BlockSpec(memory_space=pl.ANY)] * 3,
        out_specs=pl.BlockSpec(memory_space=pl.ANY),
        out_shape=jax.ShapeDtypeStruct((G, WS, WR, D), q.dtype),
        scratch_shapes=[
            pltpu.VMEM((R, C, Sq, D), q.dtype),
            pltpu.VMEM((R, C, Sk, D), k.dtype),
            pltpu.VMEM((R, C, Sk, D), v.dtype),
            pltpu.VMEM((BH * Sq, D), q.dtype),
            pltpu.SemaphoreType.DMA((R * 3,)),
            pltpu.SemaphoreType.DMA((1,)),
        ],
        compiler_params=pltpu.CompilerParams(
            vmem_limit_bytes=120 * 1024 * 1024,
        ),
    )(q.reshape(BH, Sq, D), k.reshape(BH, Sk, D), v.reshape(BH, Sk, D))
    return out.reshape(B, H, Sq, D)
```

```python
import jax
import jax.numpy as jnp
import jax.experimental.pallas as pl
import jax.experimental.pallas.tpu as pltpu

_LOG2E = 1.4426950408889634

_C = 8
_R = 4
_L = 2
_RUN = 128
_OFF = 104
_NK = 3
_NSW = 9
_PRE = 40
_PACE = 10
_PSPLIT = (0, 128, 256, 288)


def _ranges(xs):
    out = []
    for x in xs:
        if out and out[-1][1] == x:
            out[-1][1] = x + 1
        else:
            out.append([x, x + 1])
    return out


def _mo(x, m=8):
    return x if isinstance(x, int) else pl.multiple_of(x, m)


@jax.jit
def pallas_standalone__mha_softmax__near_ridge_kernel(
    q: jax.Array,
    k: jax.Array,
    v: jax.Array,
):
    B, H, Sq, D = q.shape
    Sk = k.shape[2]
    BH = B * H
    C, R, L, RUN, OFF, NK, NSW = _C, _R, _L, _RUN, _OFF, _NK, _NSW
    assert (Sq, Sk, D) == (288, 512, 128) and BH % (4 * C) == 0
    assert (BH * Sq) % (NSW * RUN) == 0 and 96 <= OFF < RUN and OFF % 16 == 8
    N = BH // C
    W0 = N - L
    NP = 2 + NK
    TAIL = RUN - OFF
    QR, QPAD = 4 * Sq, 16
    KOFF = QPAD + QR + QPAD
    AP = Sk - OFF
    LW = BH * Sq // (NSW * RUN)
    SL = LW * RUN
    CROW = NSW * SL
    scale = (D ** -0.5) * _LOG2E

    late = {LW - 1}
    for a in range(W0, N):
        for j in range(C):
            lo, hi = (j * N + a) * Sq, (j * N + a + 1) * Sq
            for run in range((lo - OFF) // RUN, (hi - 1 - OFF) // RUN + 1):
                late.add(run % LW)
    ready = [s for s in range(LW) if s not in late]
    late = sorted(late)

    def kernel_function(q_hbm, k_hbm, v_hbm, o_hbm, xb, vb, ob3, pace,
                        sin, sx, sout):
        ob = ob3.reshape((NSW + 1) * SL, D)
        every = pl.ds(0, C)

        def q_run(x, slot, t, js, n=RUN, sem=None):
            u = 9 * (x // 4) + 2 * slot + t
            return pltpu.make_async_copy(
                q_hbm.at[js, pl.ds(_mo(OFF + RUN * u), n)],
                xb.at[js, pl.ds(_mo(QPAD + RUN * (2 * slot + t)), n)],
                sin.at[slot * 4] if sem is None else sem)

        def k_run(x, slot, r, js, n=RUN):
            return pltpu.make_async_copy(
                k_hbm.at[js, pl.ds(_mo(OFF + Sk * x + RUN * r), n)],
                xb.at[js, pl.ds(_mo(KOFF + Sk * slot + RUN * r), n)],
                sin.at[slot * 4 + 1])

        def v_run(x, slot, r, js, n=RUN, sem=None):
            return pltpu.make_async_copy(
                v_hbm.at[js, pl.ds(_mo(OFF + Sk * x + RUN * r), n)],
                vb.at[js, pl.ds(_mo(Sk * slot + RUN * r), n)],
                sin.at[slot * 4 + (3 if r >= 2 else 2)] if sem is None else sem)

        def single(x, slot, w):
            kind, j = w // C, w % C
            if kind < 2:
                return q_run(x, slot, kind, j)
            if kind < 4:
                i = w - 2 * C
                return k_run(x, slot, i % 2, i // 2)
            return k_run(x, slot, kind - 2, j)

        def wait(region, sem):
            pltpu.make_async_copy(region, region, sem).wait()

        def wait_step(slot, last=False):
            wait(xb.at[every, pl.ds(_mo(QPAD + 2 * RUN * slot), 2 * RUN)],
                 sin.at[slot * 4])
            wait(xb.at[every, pl.ds(_mo(KOFF + Sk * slot),
                                    3 * RUN + (TAIL if last else RUN))],
                 sin.at[slot * 4 + 1])
            wait(vb.at[every, pl.ds(_mo(Sk * slot), 2 * RUN)],
                 sin.at[slot * 4 + 2])
            wait(vb.at[every, pl.ds(_mo(Sk * slot + (3 if last else 2) * RUN),
                                    TAIL if last else 2 * RUN)],
                 sin.at[slot * 4 + 3])

        def wait_q_extra(last=False):
            wait(xb.at[every, pl.ds(QPAD + 8 * RUN, TAIL if last else RUN)],
                 sx.at[0])

        def v_final():
            return v_run(N - 1, 3, 2, every, sem=sx.at[1])

        def o_col(r0, n):
            return pltpu.make_async_copy(
                ob3.at[pl.ds(0, NSW), pl.ds(r0, n)],
                o_hbm.at[:, pl.ds(r0, n)], sout.at[0])

        def write_back(cols):
            def start(s, carry):
                o_col(_mo(OFF + s * RUN), RUN).start()
                return carry

            for lo, hi in _ranges(cols):
                if min(hi, LW - 1) > lo:
                    jax.lax.fori_loop(lo, min(hi, LW - 1), start, 0)
                if hi == LW:
                    o_col(SL - TAIL, TAIL).start()
                    o_col(0, OFF).start()

        lead = [
            pltpu.make_async_copy(
                q_hbm.at[every, pl.ds(0, OFF)],
                xb.at[every, pl.ds(QPAD + QR - OFF, OFF)], sx.at[1]),
            pltpu.make_async_copy(
                k_hbm.at[every, pl.ds(0, OFF)],
                xb.at[every, pl.ds(KOFF + Sk * (R - 1) + AP, OFF)], sx.at[2]),
            pltpu.make_async_copy(
                v_hbm.at[every, pl.ds(0, OFF)],
                vb.at[every, pl.ds(Sk * (R - 1) + AP, OFF)], sx.at[3]),
        ]
        for cp in lead:
            cp.start(priority=1)
        for x in range(L):
            if x > 0:
                for t in range(2):
                    q_run(x, x, t, every).start(priority=1)
            for r in range(0 if x > 0 else NK, 4):
                k_run(x, x, r, every).start(priority=1)
            for r in (0, 2):
                v_run(x, x, r, every, 2 * RUN).start(priority=1)

        scale_bits = pltpu.bitcast(
            jnp.full((8, D), scale, jnp.float32), jnp.bfloat16)
        for j in range(R):
            xb[C, pl.ds(16 * j, 16), :] = scale_bits
        ob[pl.ds(CROW, 16), :] = scale_bits
        zeros = jnp.zeros((16, D), jnp.bfloat16)
        for j in range(C):
            xb[j, pl.ds(0, QPAD), :] = zeros
            xb[j, pl.ds(QPAD + QR, QPAD), :] = zeros
            xb[j, pl.ds(KOFF + Sk * (R - 1) + AP - 8, 8), :] = zeros[:8]
            vb[j, pl.ds(Sk * (R - 1) + AP - 8, 8), :] = zeros[:8]

        tick = jnp.int32(1)
        for w in range(NP * C):
            single(0, 0, w).start(priority=0)
            tick = jax.lax.fori_loop(0, _PACE, lambda i, c: c * 3 + i, tick)
        pace[0] = tick
        for cp in lead:
            cp.wait()

        low_half = jax.lax.broadcasted_iota(jnp.int32, (8, D), 0) < 4

        def merge(lo16, hi16):
            return pltpu.bitcast(
                jnp.where(low_half, pltpu.bitcast(lo16, jnp.uint32),
                          pltpu.bitcast(hi16, jnp.uint32)), jnp.bfloat16)

        def compute(a, slot, prefetch):
            nslot = (slot + L) % R
            pslot = (slot + R - 1) % R
            issued = [1]

            def dma():
                if prefetch:
                    single(a + L, nslot, issued[0]).start(priority=0)
                    issued[0] += 1

            def row0(h):
                return pl.multiple_of((h * N + a) * Sq, 32)

            def keys(ref, base, h, lo, hi):
                own, prev, mid = base + Sk * slot, base + Sk * pslot, AP - 8
                parts = []
                if lo < mid:
                    parts.append(
                        ref[h, pl.ds(_mo(own + lo, 16), min(hi, mid) - lo), :])
                if lo <= mid < hi:
                    parts.append(merge(ref[h, pl.ds(_mo(own + mid, 16), 16), :],
                                       ref[h, pl.ds(_mo(prev + mid, 16), 16), :]))
                if hi > mid + 16:
                    s0 = max(lo, mid + 16)
                    parts.append(ref[h, pl.ds(_mo(prev + s0, 16), hi - s0), :])
                return jnp.concatenate(parts, axis=0)

            q2 = QPAD + Sq * slot
            q1 = jnp.where(slot == 0, QPAD + QR - OFF, q2 - OFF)
            pending = None
            kh = keys(xb, KOFF, 0, 0, Sk)
            for h in range(C):
                if h > 0:
                    dma()
                qs = [xb[h, pl.ds(_mo(q1), OFF - 8), :],
                      merge(xb[h, pl.ds(_mo(q1 + OFF - 8), 16), :],
                            xb[h, pl.ds(_mo(q2 - 8), 16), :]),
                      xb[h, pl.ds(_mo(q2 + 8), RUN - OFF - 8), :]]
                dma()
                qs.append(xb[h, pl.ds(_mo(q2 + RUN - OFF), RUN), :])
                dma()
                qs.append(xb[h, pl.ds(_mo(q2 + 2 * RUN - OFF), Sq - 2 * RUN), :])
                vh = keys(vb, 0, h, 0, Sk)
                s = jax.lax.dot_general(
                    jnp.concatenate(qs, axis=0), kh, (((1,), (1,)), ((), ())),
                    preferred_element_type=jnp.float32)
                d = s - jnp.max(s, axis=-1, keepdims=True)
                if pending is not None:
                    ob[pl.ds(row0(h - 1), Sq), :] = pending
                ps = []
                kparts = {}
                for t, (lo, hi) in enumerate(zip(_PSPLIT[:-1], _PSPLIT[1:])):
                    if t == 0:
                        bits = ob[pl.ds(CROW, 16), :]
                    else:
                        if h + 1 < C:
                            off = RUN // 2 if t == 1 else 0
                            for r in range(4):
                                kparts[(r, off)] = keys(
                                    xb, KOFF, h + 1, r * RUN + off,
                                    r * RUN + off + RUN // 2)
                        dma()
                        bits = xb[C, pl.ds(_mo(16 * slot, 16), 16), :]
                    cv = pltpu.bitcast(bits, jnp.float32)
                    cv = jnp.concatenate([cv] * (Sk // D), axis=1)
                    cv = jnp.concatenate([cv] * ((hi - lo) // 8), axis=0)
                    ps.append(jnp.exp2(d[lo:hi] * cv))
                p = jnp.concatenate(ps, axis=0)
                if h + 1 < C:
                    kh = jnp.concatenate(
                        [kparts[(r, off)] for r in range(4)
                         for off in (0, RUN // 2)], axis=0)
                l = jnp.sum(p, axis=-1, keepdims=True)
                o = jnp.dot(p.astype(jnp.bfloat16), vh,
                            preferred_element_type=jnp.float32)
                inv = pl.reciprocal(l, approx=True)
                inv = inv * (2.0 - l * inv)
                pending = (o * inv).astype(ob.dtype)
            ob[pl.ds(row0(C - 1), Sq), :] = pending
            assert (not prefetch) or issued[0] == NP * C

        def step(a, carry):
            slot = a % R
            nxt = a + L
            nslot = nxt % R

            @pl.when(nxt < N - 1)
            def _():
                @pl.when(nslot == 3)
                def _():
                    q_run(nxt, 3, 2, every, sem=sx.at[0]).start(priority=1)

                for r in range(NK, 4):
                    k_run(nxt, nslot, r, every).start(priority=1)
                for r in (0, 2):
                    v_run(nxt, nslot, r, every, 2 * RUN).start(priority=1)

            @pl.when(nxt == N - 1)
            def _():
                q_run(N - 1, 3, 2, every, TAIL, sx.at[0]).start(priority=1)
                for r in range(NK, 3):
                    k_run(N - 1, 3, r, every).start(priority=1)
                k_run(N - 1, 3, 3, every, TAIL).start(priority=1)
                v_run(N - 1, 3, 3, every, TAIL).start(priority=1)
                v_run(N - 1, 3, 0, every, 2 * RUN).start(priority=1)
                v_final().start(priority=1)

            @pl.when(slot == 3)
            def _():
                wait_q_extra()

            single(nxt, nslot, 0).start(priority=0)
            wait_step(slot)
            compute(a, slot, True)
            return carry

        jax.lax.fori_loop(0, W0, step, 0)

        for x in range(W0, N):
            if x % R == 3:
                wait_q_extra(last=(x == N - 1))
            wait_step(x % R, last=(x == N - 1))
        write_back(ready[:_PRE])
        v_final().wait()

        def last_steps(a, carry):
            compute(a, a % R, False)
            return carry

        jax.lax.fori_loop(W0, N, last_steps, 0)
        write_back(ready[_PRE:])
        write_back(late)
        o_col(0, SL).wait()

    out = pl.pallas_call(
        kernel_function,
        in_specs=[pl.BlockSpec(memory_space=pl.ANY)] * 3,
        out_specs=pl.BlockSpec(memory_space=pl.ANY),
        out_shape=jax.ShapeDtypeStruct((NSW, SL, D), q.dtype),
        scratch_shapes=[
            pltpu.VMEM((C + 1, KOFF + R * Sk, D), q.dtype),
            pltpu.VMEM((C, R * Sk, D), v.dtype),
            pltpu.VMEM((NSW + 1, SL, D), q.dtype),
            pltpu.SMEM((1,), jnp.int32),
            pltpu.SemaphoreType.DMA((R * 4,)),
            pltpu.SemaphoreType.DMA((4,)),
            pltpu.SemaphoreType.DMA((1,)),
        ],
        compiler_params=pltpu.CompilerParams(
            vmem_limit_bytes=100 * 1024 * 1024,
            disable_bounds_checks=True,
            disable_semaphore_checks=True,
        ),
    )(q.reshape(C, N * Sq, D), k.reshape(C, N * Sk, D), v.reshape(C, N * Sk, D))
    return out.reshape(B, H, Sq, D)
```
